```python
import jax
import jax.numpy as jnp

def _softmax(x, axis=-1):
    return jax.nn.softmax(x, axis=axis)
def _gelu(x):
    return jax.nn.gelu(x, approximate=True)
def _silu(x):
    return jax.nn.silu(x)
def _sigmoid(x):
    return jax.nn.sigmoid(x)
def _layernorm(x, axis=-1, eps=1e-5):
    m = jnp.mean(x, axis=axis, keepdims=True)
    v = jnp.var(x, axis=axis, keepdims=True)
    return (x - m) / jnp.sqrt(v + eps)
def _scatter_add(tgt, idx, src, axis=0):
    return tgt.at[idx].add(src)
def _segment_sum(src, seg, n):
    return jax.ops.segment_sum(src, seg, n)
class _Rng:
    def __init__(self, key):
        self._k = key
    def _next(self):
        self._k, sub = jax.random.split(self._k)
        return sub
    def normal(self, shape):
        return jax.random.normal(self._next(), shape, dtype=jnp.bfloat16)
    def randint(self, lo, hi, shape):
        return jax.random.randint(self._next(), shape, lo, hi, dtype=jnp.int32)
    def uniform(self, shape, lo=0.0, hi=1.0):
        return jax.random.uniform(self._next(), shape, jnp.bfloat16, lo, hi)
    def permutation(self, n):
        return jax.random.permutation(self._next(), n)


kernel_name = 'sequential_preLN__sliding_block_cached__moe_arch_mod__decode'

def setup_inputs():
    _rng = _Rng(jax.random.key(int.from_bytes(__import__("os").urandom(4), "little")))
    _w = (lambda a: (lambda t: t.astype(jnp.bfloat16) if jnp.issubdtype(t.dtype, jnp.floating) else t)(jnp.asarray(a)))
    def _A_setup():
        B, Sq, D = 1, 1, 640
        Hq, Hkv, Sk, Dh = 32, 32, 32768, 192
        assert Hq % Hkv == 0, (Hq, Hkv)
        return {
            "x": _w((lambda *s: _rng.normal(s) * 0.05)(B, Sq, D)),
            "k_cache": _w((lambda *s: _rng.normal(s) * 0.05)(B, Hkv, Sk, Dh)),
            "v_cache": _w((lambda *s: _rng.normal(s) * 0.05)(B, Hkv, Sk, Dh)),
            "wq": _w((lambda *s: _rng.normal(s) * 0.05)(D, Hq * Dh) * (D ** -0.5)),
            "wo": _w((lambda *s: _rng.normal(s) * 0.05)(Hq * Dh, D) * ((Hq * Dh) ** -0.5)),
        }
    _A_in = _A_setup()

    def _B_setup():
        B, S, D, F, C = 1, 1, 640, 1536, 1
        return {
            "x": _w((lambda *s: _rng.normal(s) * 0.05)(B, S, D)),
            "w_r": _w((lambda *s: _rng.normal(s) * 0.05)(D)),
            "w_gate": _w((lambda *s: _rng.normal(s) * 0.05)(D, F)),
            "w_up": _w((lambda *s: _rng.normal(s) * 0.05)(D, F)),
            "w_down": _w((lambda *s: _rng.normal(s) * 0.05)(F, D)),
        }
    _B_in = _B_setup()

    return {
        "A_x": _A_in["x"],
        "A_k_cache": _A_in["k_cache"],
        "A_v_cache": _A_in["v_cache"],
        "A_wq": _A_in["wq"],
        "A_wo": _A_in["wo"],
        "B_x": _B_in["x"],
        "B_w_r": _B_in["w_r"],
        "B_w_gate": _B_in["w_gate"],
        "B_w_up": _B_in["w_up"],
        "B_w_down": _B_in["w_down"],
    }

def reference(A_x, A_k_cache, A_v_cache, A_wq, A_wo, B_x, B_w_r, B_w_gate, B_w_up, B_w_down):
    def _A_ref(x, k_cache, v_cache, wq, wo):
        B, Sq, D = x.shape
        Hq, Dh = 32, 192
        Hkv, Sk = k_cache.shape[1], k_cache.shape[2]
        W = min(4096, max(256, Sk // 4))
        rep = Hq // Hkv
        q = (lambda x, *d: x.transpose(*d))((x @ wq).reshape(B, Sq, Hq, Dh), 0, 2, 1, 3)
        k = jnp.repeat(k_cache[:, :, Sk - W:, :], rep, axis=1)
        v = jnp.repeat(v_cache[:, :, Sk - W:, :], rep, axis=1)
        scores = jnp.einsum("bhqd,bhkd->bhqk", q, k) * (Dh ** -0.5)
        p = _softmax(scores, axis=-1)
        o = jnp.einsum("bhqk,bhkd->bhqd", p, v)
        return (lambda x, *d: x.transpose(*d))(o, 0, 2, 1, 3).reshape(B, Sq, Hq * Dh) @ wo

    def _B_ref(x, w_r, w_gate, w_up, w_down):
        B, S, D = x.shape
        C = 1
        r = x @ w_r
        idx = jnp.argsort(-r, axis=-1)[:, :C]
        idx_e = jnp.repeat(idx.reshape(B, C, 1), D, axis=2)
        x_sel = jnp.take_along_axis(x, idx_e, axis=1)
        g = _silu(x_sel @ w_gate)
        u = x_sel @ w_up
        y = (g * u) @ w_down
        r_sel = _sigmoid(jnp.take_along_axis(r, idx, axis=1))
        y = y * r_sel.reshape(B, C, 1)
        b_off = (jnp.arange(B) * S).reshape(B, 1)
        flat_idx = (idx + b_off).reshape(B * C)
        zero = (x * 0.0).reshape(B * S, D)
        upd = _scatter_add(zero, flat_idx, y.reshape(B * C, D), axis=0)
        return x + upd.reshape(B, S, D)

    x = A_x
    h = x + _A_ref(_layernorm(x, axis=-1), A_k_cache, A_v_cache, A_wq, A_wo)
    h2 = h + _B_ref(_layernorm(h, axis=-1), B_w_r, B_w_gate, B_w_up, B_w_down)
    return h2
```

```python
import jax
import jax.numpy as jnp
from jax import lax
import jax.experimental.pallas as pl
import jax.experimental.pallas.tpu as pltpu

EPS = 1e-5
H, Dh, D, F, W = 32, 192, 640, 1536, 4096
K_, V_, Q_, O_, G_, U_, D_ = range(7)


def zip2(A, B):
    out = []
    for j in range(max(len(A), len(B))):
        if j < len(A):
            out.append((A[j], 0))
        if j < len(B):
            out.append((B[j], 1))
    return out


def alt(l):
    return [(p, i % 2) for i, p in enumerate(l)]


def part(l, i, n):
    return l[len(l) * i // n:len(l) * (i + 1) // n]


def _layernorm(x):
    m = jnp.mean(x, axis=-1, keepdims=True)
    d = x - m
    v = jnp.mean(d * d, axis=-1, keepdims=True)
    return d / jnp.sqrt(v + EPS)


def make(name="k2", look=2, gq=16, go=6, nkv=3, dkv=35, lead=27, nsmall=7,
         dcuts=(128, 256, 320, 384), tail_split=(0.45, 0.65),
         lag=27, extra=0, compute=True, sem_checks=False, bounds=False, scopes=False, xpos=40):
    nbuf = look + 1
    gg, gd = 4, 4
    cuts = (0,) + tuple(dcuts)
    ncut = len(dcuts)

    q = [(Q_, g, 4, r, 8, c, 512) for r in range(0, D // gq, 8) for c in range(0, H * Dh, 512)
         for g in range(0, gq, 4)]
    qa, qb = q[0::2], q[1::2]
    first = [(p, 1) for p in qb[:lead]] + zip2(qa, qb[lead:])
    kk = [(K_, 0, 1, r, 8 * nkv, c, 512) for c in range(0, W, 512) for r in range(0, Dh, 8 * nkv)]
    vv = [(V_, 0, 1, r, 8 * nkv, c, 512) for c in range(0, W, 512) for r in range(0, Dh, 8 * nkv)]
    orows = H * Dh // go // H
    wo = [(O_, g, 3, r, 8, 0, D) for r in range(0, orows, 8) for g in range(0, go, 3)]
    period = zip2(kk, vv[dkv:] + vv[:dkv]) + alt(wo)
    g_ = [(G_, 0, gg, r, 8, c, 512) for r in range(0, D // gg, 8) for c in range(0, F, 512)]
    u_ = [(U_, 0, gg, r, 8, c, 512) for r in range(0, D // gg, 8) for c in range(0, F, 512)]
    nrow = F // gd // 8
    big = [(D_, 0, gd, 8 * r, 8, 0, D) for r in range(nrow - nsmall)]
    small = [(D_, g, 1, 8 * r, 8, 0, D) for r in range(nrow - nsmall, nrow) for g in range(gd)]
    nu = (lag - 1) // 2
    head_ = [x for p in zip(g_[:nu], u_[:nu]) for x in p]
    A = head_ + g_[nu:]
    B = u_[nu:]
    na = (len(A) + len(B) + len(big) + len(small) + extra) // 2 - len(A)
    nb = len(big) - na
    A += big[0:2 * nb:2] + big[2 * nb:]
    B += big[1:2 * nb:2] + small
    tail = zip2(A, B)

    class _Null:
        def __enter__(self):
            return None

        def __exit__(self, *a):
            return False

    def scope(n):
        return jax.named_scope(n) if scopes else _Null()

    def kernel(x_hbm, kt_hbm, vt_hbm, wq_hbm, wo_hbm, wr_hbm, wg_hbm, wu_hbm, wd_hbm,
               o_ref,
               x_s, wr_s, wq_s, wo_s, wg_s, wu_s, wd_s, k_s, v_s, q_s, p_s, o_s, sems):
        Sk = kt_hbm.shape[-1]
        f32, bf16 = jnp.float32, jnp.bfloat16
        SQ, SO, SG, SU, SX, SR, SD = (2 * nbuf + i for i in range(7))

        def start(piece, prio, h=None, slot=None):
            a, g, ng, r, nr, c, nc = piece
            if a in (K_, V_):
                hbm, buf, s0 = (kt_hbm, k_s, 0) if a == K_ else (vt_hbm, v_s, nbuf)
                src = hbm.at[0, h, pl.ds(r, nr), pl.ds(Sk - W + c, nc)]
                dst = buf.at[slot, pl.ds(r, nr), pl.ds(c, nc)]
                sem = sems.at[s0 + slot]
            else:
                hbm, buf, si = {Q_: (wq_hbm, wq_s, SQ), O_: (wo_hbm, wo_s, SO), G_: (wg_hbm, wg_s, SG),
                                U_: (wu_hbm, wu_s, SU), D_: (wd_hbm, wd_s, SD)}[a]
                if a == O_:
                    r = h * orows + r
                    if not isinstance(h, int):
                        r = pl.multiple_of(r, 8)
                if a == D_:
                    si += [j for j in range(ncut) if cuts[j] <= r and r + nr <= cuts[j + 1]][0]
                idx = (pl.ds(g, ng), pl.ds(r, nr), pl.ds(c, nc))
                src, dst, sem = hbm.at[idx], buf.at[idx], sems.at[si]
            pltpu.make_async_copy(src, dst, sem).start(priority=prio)

        def done(dst, si):
            pltpu.make_async_copy(dst, dst, sems.at[si]).wait()

        x_cp = pltpu.make_async_copy(x_hbm, x_s, sems.at[SX])
        wr_cp = pltpu.make_async_copy(wr_hbm, wr_s, sems.at[SR])

        with scope("prologue"):
            for n, (piece, prio) in enumerate(first):
                start(piece, prio)
                if n == xpos:
                    x_cp.start()
                    wr_cp.start(priority=1)
            for h in range(look - 1):
                for piece, prio in period:
                    start(piece, prio, h, h)

        with scope("q"):
            x_cp.wait()
            x = x_s[0].astype(f32)
            xn = jnp.broadcast_to(_layernorm(x), (8, D)).astype(bf16)
            done(wq_s, SQ)
            QC = 2 * Dh
            for c in range(H // 2):
                for piece, prio in part(period, c, H // 2):
                    start(piece, prio, look - 1, look - 1)
                if compute:
                    w = wq_s[:, :, c * QC:(c + 1) * QC].reshape(D, QC)
                    q2 = jnp.dot(xn, w, preferred_element_type=f32)
                    q_s[2 * c] = q2[:, :Dh]
                    q_s[2 * c + 1] = q2[:, Dh:]

        scale = Dh ** -0.5
        NS = Dh // 16 + 2

        def head(h, slot, issue):
            done(k_s.at[slot], slot)
            issue(0)
            if compute:
                s = jnp.dot(q_s[h].astype(bf16), k_s[slot], preferred_element_type=f32) * scale
            issue(1)
            if compute:
                m = jnp.max(s, axis=-1, keepdims=True)
                e = jnp.exp(s - m)
                l = jnp.sum(e, axis=-1, keepdims=True)
                p_s[...] = e
                inv = 1.0 / l
            done(v_s.at[slot], nbuf + slot)
            parts = []
            for r in range(Dh // 16):
                issue(r + 2)
                if not compute:
                    continue
                a0 = jnp.zeros((8, 128), f32)
                a1 = jnp.zeros((8, 128), f32)
                for j in range(W // 128):
                    vv = v_s[slot, r * 16:(r + 1) * 16, j * 128:(j + 1) * 128].astype(f32)
                    pp = p_s[:, j * 128:(j + 1) * 128]
                    a0 = a0 + vv[:8] * pp
                    a1 = a1 + vv[8:] * pp
                parts += [a0, a1]
            if compute:
                parts += [jnp.zeros((64, 128), f32)]
                pt = jnp.concatenate(parts, axis=0).T
                o = jnp.sum(pt, axis=0, keepdims=True)
                o_s[h] = o * inv
        def step(h, slot):
            nslot = jnp.where(slot == 0, nbuf - 1, slot - 1)

            def issue(i):
                for piece, prio in part(period, i, NS):
                    start(piece, prio, h + look, nslot)
            with scope("head"):
                head(h, slot, issue)
            return jnp.where(slot == nbuf - 1, 0, slot + 1)

        lax.fori_loop(0, H - look, step, 0)

        nt = len(tail)
        marks = [0] + [int(nt * f) // 2 * 2 for f in tail_split] + [nt]
        for t in range(look):
            h = H - look + t
            tl = tail[marks[t]:marks[t + 1]]

            def issue(i, tl=tl):
                for piece, prio in part(tl, i, NS):
                    start(piece, prio)
            with scope("tailhead"):
                head(h, h % nbuf, issue)

        with scope("oproj"):
            done(wo_s, SO)
            tl = tail[marks[look]:]
            acc = jnp.zeros((8, D), f32)
            rows = H * Dh // go
            for h in range(H):
                for piece, prio in part(tl, h, H):
                    start(piece, prio)
                if compute:
                    lo, hi = h * Dh, (h + 1) * Dh
                    if lo // rows == (hi - 1) // rows:
                        w = wo_s[lo // rows, lo % rows:lo % rows + Dh, :]
                    else:
                        cut = (hi - 1) // rows * rows
                        w = jnp.concatenate([wo_s[lo // rows, lo % rows:, :], wo_s[cut // rows, :hi - cut, :]],
                                            axis=0)
                    acc = acc + jnp.dot(o_s[h][:, :Dh].astype(bf16), w, preferred_element_type=f32)

        with scope("ln"):
            hres = x + acc[:1]
            hn = _layernorm(hres)
            wr_cp.wait()
            wr = wr_s[...].astype(f32).reshape(1, D)
            gate = jax.nn.sigmoid(jnp.sum(hn * wr, axis=-1, keepdims=True))
            hb = jnp.broadcast_to(hn, (8, D)).astype(bf16)
        with scope("gu"):
            done(wg_s, SG)
            g = jnp.dot(hb, wg_s[...].reshape(D, F), preferred_element_type=f32)
            done(wu_s, SU)
            u = jnp.dot(hb, wu_s[...].reshape(D, F), preferred_element_type=f32)
            gu = (g * jax.nn.sigmoid(g) * u).astype(bf16)
            base = hres + hn
            lhs = []
            for c in range(ncut):
                lo, hi = cuts[c], cuts[c + 1]
                lhs.append(jnp.concatenate(
                    [gu[:, i * (F // gd) + lo:i * (F // gd) + hi] for i in range(gd)], axis=1))
        y = jnp.zeros((8, D), f32)
        for c in range(ncut):
            lo, hi = cuts[c], cuts[c + 1]
            with scope("dwait"):
                done(wd_s.at[:, pl.ds(lo, hi - lo)], SD + c)
            with scope("down"):
                w = wd_s[:, lo:hi, :].reshape(gd * (hi - lo), D)
                y = y + jnp.dot(lhs[c], w, preferred_element_type=f32)
        out = base + y[:1] * gate
        o_ref[0] = out.astype(o_ref.dtype)

    def fn(A_x, A_k_cache, A_v_cache, A_wq, A_wo, B_x, B_w_r, B_w_gate, B_w_up, B_w_down):
        kt = jnp.transpose(A_k_cache, (0, 1, 3, 2))
        vt = jnp.transpose(A_v_cache, (0, 1, 3, 2))
        grp = lambda a, n: a.reshape(n, a.shape[0] // n, a.shape[1])
        wq, wo = grp(A_wq, gq), grp(A_wo, go)
        wg, wu, wd = grp(B_w_gate, gg), grp(B_w_up, gg), grp(B_w_down, gd)
        like = lambda a: pltpu.VMEM(a.shape, a.dtype)
        return pl.pallas_call(
            kernel, name=name,
            out_shape=jax.ShapeDtypeStruct(A_x.shape, A_x.dtype),
            in_specs=[pl.BlockSpec(memory_space=pl.ANY)] * 9,
            scratch_shapes=[
                like(A_x), like(B_w_r), like(wq), like(wo), like(wg), like(wu), like(wd),
                pltpu.VMEM((nbuf, Dh, W), A_k_cache.dtype),
                pltpu.VMEM((nbuf, Dh, W), A_v_cache.dtype),
                pltpu.VMEM((H, 8, Dh), jnp.float32),
                pltpu.VMEM((8, W), jnp.float32),
                pltpu.VMEM((H, 8, 256), jnp.float32),
                pltpu.SemaphoreType.DMA((2 * nbuf + 6 + ncut,)),
            ],
            compiler_params=pltpu.CompilerParams(
                vmem_limit_bytes=100 * 2**20,
                disable_bounds_checks=not bounds, disable_semaphore_checks=not sem_checks),
        )(A_x, kt, vt, wq, wo, B_w_r, wg, wu, wd)
    return fn


pallas_sequential_preLN__sliding_block_cached__moe_arch_mod__decode_kernel = jax.jit(make())
```

```python
import jax
import jax.numpy as jnp
from jax import lax
import jax.experimental.pallas as pl
import jax.experimental.pallas.tpu as pltpu

EPS = 1e-5
H, Dh, D, F, W = 32, 192, 640, 1536, 4096
K_, V_, Q_, O_, G_, U_, D_ = range(7)


def part(l, i, n):
    return l[len(l) * i // n:len(l) * (i + 1) // n]


def _layernorm(x):
    m = jnp.mean(x, axis=-1, keepdims=True)
    d = x - m
    v = jnp.mean(d * d, axis=-1, keepdims=True)
    return d / jnp.sqrt(v + EPS)


def make(name="k3", look=2, lag=26, nsmall=1, dcuts=(128, 256, 320, 352, 368, 384), nvpu=3,
         flat=True, mirror=True, ahead=84, n_oproj=72, n_last=24,
         compute=True, sem_checks=False, bounds=False, scopes=False, xpos=40, flags=None):
    nbuf = look + 2
    gg, gd = 4, 4
    cuts = (0,) + tuple(dcuts)
    ncut = len(dcuts)

    def sweep(a, groups, step, col, h=None):
        return [((a, g, 1, col, h), (a, g + 1, step - 1, col, h)) for g in range(0, groups, step)]

    gq = 15 if flat else 16
    go = 15 if flat else 6
    if flat:
        first = [p for c in range(64) for p in sweep(Q_, gq, 5, c)]
        wo = [p for c in range(64) for p in sweep(O_, go, 5, c)]
    else:
        first = [p for c in range(60) for p in sweep(Q_, gq, 4, c)]
        wo = [p for c in range(128) for p in sweep(O_, go, 6, c)]
    heads = [p for h in range(H) for a in (K_, V_) for c in range(8) for p in sweep(a, 24, 6, c, h)]
    gu = []
    for c in range(60):
        gu += sweep(G_, gg, 4, c)
        gu += [((U_, 3, 1, c, None), (U_, 0, 3, c, None))] if mirror else sweep(U_, gg, 4, c)
    nrow = F // gd // 8
    wd = [p for c in range(nrow - nsmall) for p in sweep(D_, gd, 4, c)]
    small = [(D_, g, 1, (c, t), None) for c in range(nrow - nsmall, nrow) for t in range(D // 128)
             for g in range(gd)]
    pairs = first + heads + wo + gu + wd
    A = [p[0] for p in pairs]
    B = [p[1] for p in pairs] + small
    stream = [(b, 1) for b in B[:lag]]
    for j in range(max(len(A), len(B) - lag)):
        if j < len(A):
            stream.append((A[j], 0))
        if j + lag < len(B):
            stream.append((B[j + lag], 1))
    per = 2 * len(heads) // H
    s0 = lag + 2 * len(first)
    nloop = H - look - 1
    pre = stream[:s0 + (look - 1) * per]
    during_q = stream[len(pre):s0 + look * per]
    body = stream[s0 + look * per:s0 + (look + 1) * per]
    tail = stream[s0 + (look + nloop) * per:]

    class _Null:
        def __enter__(self):
            return None

        def __exit__(self, *a):
            return False

    def scope(n):
        return jax.named_scope(n) if scopes else _Null()

    def kernel(x_hbm, kt_hbm, vt_hbm, wq_hbm, wo_hbm, wr_hbm, wg_hbm, wu_hbm, wd_hbm,
               o_ref,
               x_s, wr_s, wq_s, wo_s, wg_s, wu_s, wd_s, k_s, v_s, q_s, p_s, o_s, sems):
        Sk = kt_hbm.shape[-1]
        f32, bf16 = jnp.float32, jnp.bfloat16
        SQ, SO, SG, SU, SX, SR, SD = (2 * nbuf + i for i in range(7))

        def start(piece, prio, i=0):
            a, g, ng, c, h = piece
            si = 0
            if a in (K_, V_):
                hbm, buf, s0_ = (kt_hbm, k_s, 0) if a == K_ else (vt_hbm, v_s, nbuf)
                h = h + i
                slot = h & (nbuf - 1)
                src = hbm.at[0, h, pl.ds(8 * g, 8 * ng), pl.ds(Sk - W + 512 * c, 512)]
                dst = buf.at[slot, pl.ds(8 * g, 8 * ng), pl.ds(512 * c, 512)]
                sem = sems.at[s0_ + slot]
            else:
                hbm, buf, si = {Q_: (wq_hbm, wq_s, SQ), O_: (wo_hbm, wo_s, SO), G_: (wg_hbm, wg_s, SG),
                                U_: (wu_hbm, wu_s, SU), D_: (wd_hbm, wd_s, SD)}[a]
                if a in (Q_, O_) and flat:
                    idx = (pl.ds(g, ng), pl.ds(4 * c, 4))
                elif a == Q_:
                    idx = (pl.ds(g, ng), pl.ds(8 * (c // 12), 8), pl.ds(512 * (c % 12), 512))
                elif a in (G_, U_):
                    idx = (pl.ds(g, ng), pl.ds(8 * (c // 3), 8), pl.ds(512 * (c % 3), 512))
                elif isinstance(c, tuple):
                    idx = (pl.ds(g, ng), pl.ds(8 * c[0], 8), pl.ds(128 * c[1], 128))
                    c = c[0]
                else:
                    idx = (pl.ds(g, ng), pl.ds(8 * c, 8))
                if a == D_:
                    si += [j for j in range(ncut) if cuts[j] <= 8 * c < cuts[j + 1]][0]
                src, dst, sem = hbm.at[idx], buf.at[idx], sems.at[si]
            pltpu.make_async_copy(src, dst, sem).start(priority=prio)

        def issue(l, i=0):
            for piece, prio in l:
                start(piece, prio, i)

        def done(dst, si):
            pltpu.make_async_copy(dst, dst, sems.at[si]).wait()

        def slab(ref, ncol, r0, r1, j):
            t = [i * ncol + j for i in range(r0 // 8, r1 // 8)]
            return jnp.concatenate([ref[n // 256, n % 256] for n in t], axis=0)

        x_cp = pltpu.make_async_copy(x_hbm, x_s, sems.at[SX])
        wr_cp = pltpu.make_async_copy(wr_hbm, wr_s, sems.at[SR])

        with scope("prologue"):
            issue(pre[:xpos])
            x_cp.start()
            wr_cp.start(priority=1)
            issue(pre[xpos:])

        with scope("q"):
            x_cp.wait()
            x = x_s[0].astype(f32)
            xn = jnp.broadcast_to(_layernorm(x), (8, D)).astype(bf16)
            done(wq_s, SQ)
            QC = 2 * Dh
            for c in range(H // 2):
                issue(part(during_q, c, H // 2))
                if compute:
                    if flat:
                        w = jnp.concatenate([slab(wq_s, H * Dh // 128, 0, D, 3 * c + j) for j in range(3)], axis=1)
                    else:
                        w = wq_s[:, :, c * QC:(c + 1) * QC].reshape(D, QC)
                    q2 = jnp.dot(xn, w, preferred_element_type=f32)
                    q_s[2 * c] = q2[:, :Dh]
                    q_s[2 * c + 1] = q2[:, Dh:]

        scale = Dh ** -0.5
        NS = Dh // 16 + 2

        def head(h, copies, i=0):
            slot = h & (nbuf - 1)
            done(k_s.at[slot], slot)
            issue(part(copies, 0, NS), i)
            if compute:
                s = jnp.dot(q_s[h].astype(bf16), k_s[slot], preferred_element_type=f32) * scale
            issue(part(copies, 1, NS), i)
            if compute:
                m = jnp.max(s, axis=-1, keepdims=True)
                e = jnp.exp(s - m)
                l = jnp.sum(e, axis=-1, keepdims=True)
                p_s[...] = e
                inv = 1.0 / l
            done(v_s.at[slot], nbuf + slot)
            parts = []
            for r in range(Dh // 16):
                issue(part(copies, r + 2, NS), i)
                if not compute:
                    continue
                a0 = jnp.zeros((8, 128), f32)
                a1 = jnp.zeros((8, 128), f32)
                for j in range(W // 128):
                    vv = v_s[slot, r * 16:(r + 1) * 16, j * 128:(j + 1) * 128].astype(f32)
                    pp = p_s[:, j * 128:(j + 1) * 128]
                    a0 = a0 + vv[:8] * pp
                    a1 = a1 + vv[8:] * pp
                parts += [a0, a1]
            if compute:
                parts += [jnp.zeros((64, 128), f32)]
                pt = jnp.concatenate(parts, axis=0).T
                o = jnp.sum(pt, axis=0, keepdims=True)
                o_s[h] = o * inv

        def step(h, _):
            with scope("head"):
                head(h, body, h)

        lax.fori_loop(0, nloop, step, None)

        nt = len(tail)
        m0 = max(i for i, (p, _) in enumerate(tail) if p[0] == O_) + ahead
        for t in range(look + 1):
            with scope("tailhead"):
                head(nloop + t, part(tail[:m0], t, look + 1))

        with scope("oproj"):
            done(wo_s, SO)
            tl = tail[m0:m0 + n_oproj]
            acc = jnp.zeros((8, D), f32)
            rows = H * Dh // go
            for h in range(H):
                issue(part(tl, h, H))
                if compute:
                    lo, hi = h * Dh, (h + 1) * Dh
                    if flat:
                        w = jnp.concatenate([slab(wo_s, D // 128, lo, hi, j) for j in range(D // 128)], axis=1)
                    elif lo // rows == (hi - 1) // rows:
                        w = wo_s[lo // rows, lo % rows:lo % rows + Dh, :]
                    else:
                        cut = (hi - 1) // rows * rows
                        w = jnp.concatenate([wo_s[lo // rows, lo % rows:, :], wo_s[cut // rows, :hi - cut, :]],
                                            axis=0)
                    acc = acc + jnp.dot(o_s[h][:, :Dh].astype(bf16), w, preferred_element_type=f32)

        with scope("ln"):
            hres = x + acc[:1]
            hn = _layernorm(hres)
            wr_cp.wait()
            wr = wr_s[...].astype(f32).reshape(1, D)
            gate = jax.nn.sigmoid(jnp.sum(hn * wr, axis=-1, keepdims=True))
            hb = jnp.broadcast_to(hn, (8, D)).astype(bf16)
        with scope("rest"):
            issue(tail[m0 + n_oproj:nt - n_last])
        with scope("gu"):
            done(wg_s, SG)
            issue(tail[nt - n_last:])
            g = jnp.dot(hb, wg_s[...].reshape(D, F), preferred_element_type=f32)
            done(wu_s, SU)
            u = jnp.dot(hb, wu_s[...].reshape(D, F), preferred_element_type=f32)
            gu = (g * jax.nn.sigmoid(g) * u).astype(bf16)
            base = hres + hn
            lhs = []
            nm = ncut - nvpu
            for c in range(nm):
                lo, hi = cuts[c], cuts[c + 1]
                lhs.append(jnp.concatenate(
                    [gu[:, i * (F // gd) + lo:i * (F // gd) + hi] for i in range(gd)], axis=1))
            if nvpu:
                v0 = cuts[nm]
                nv = F // gd - v0
                gf = gu.astype(f32)
                row = jnp.concatenate([gf[:1, i * (F // gd) + v0:(i + 1) * (F // gd)] for i in range(gd)]
                                      + ([jnp.zeros((1, -gd * nv % 128), f32)] if gd * nv % 128 else []), axis=1)
                gcol = jnp.broadcast_to(row, (128, row.shape[1])).T
        y = jnp.zeros((8, D), f32)
        for c in range(nm):
            lo, hi = cuts[c], cuts[c + 1]
            with scope("dwait"):
                done(wd_s.at[:, pl.ds(lo, hi - lo)], SD + c)
            with scope("down"):
                w = wd_s[:, lo:hi, :].reshape(gd * (hi - lo), D)
                y = y + jnp.dot(lhs[c], w, preferred_element_type=f32)
        out = base + y[:1] * gate
        if nvpu:
            z = jnp.zeros((8, D), f32)
            for c in range(nm, ncut):
                lo, hi = cuts[c], cuts[c + 1]
                with scope("dwait"):
                    done(wd_s.at[:, pl.ds(lo, hi - lo)], SD + c)
                with scope("vpu"):
                    for i in range(gd):
                        for r in range(lo, hi, 8):
                            k = i * nv + r - v0
                            gk = gcol[k:k + 8]
                            z = z + wd_s[i, r:r + 8, :].astype(f32) * jnp.concatenate([gk] * (D // 128), axis=1)
            out = out + jnp.sum(z, axis=0, keepdims=True) * gate
        o_ref[0] = out.astype(o_ref.dtype)

    def fn(A_x, A_k_cache, A_v_cache, A_wq, A_wo, B_x, B_w_r, B_w_gate, B_w_up, B_w_down):
        kt = jnp.transpose(A_k_cache, (0, 1, 3, 2))
        vt = jnp.transpose(A_v_cache, (0, 1, 3, 2))
        grp = lambda a, n: a.reshape(n, a.shape[0] // n, a.shape[1])

        def tiles(a):
            r, c = a.shape
            return a.reshape(r // 8, 8, c // 128, 128).transpose(0, 2, 1, 3).reshape(-1, 256, 8, 128)
        wq, wo = (tiles(A_wq), tiles(A_wo)) if flat else (grp(A_wq, gq), grp(A_wo, go))
        wg, wu, wd = grp(B_w_gate, gg), grp(B_w_up, gg), grp(B_w_down, gd)
        like = lambda a: pltpu.VMEM(a.shape, a.dtype)
        return pl.pallas_call(
            kernel, name=name,
            out_shape=jax.ShapeDtypeStruct(A_x.shape, A_x.dtype),
            in_specs=[pl.BlockSpec(memory_space=pl.ANY)] * 9,
            scratch_shapes=[
                like(A_x), like(B_w_r), like(wq), like(wo), like(wg), like(wu), like(wd),
                pltpu.VMEM((nbuf, Dh, W), A_k_cache.dtype),
                pltpu.VMEM((nbuf, Dh, W), A_v_cache.dtype),
                pltpu.VMEM((H, 8, Dh), jnp.float32),
                pltpu.VMEM((8, W), jnp.float32),
                pltpu.VMEM((H, 8, 256), jnp.float32),
                pltpu.SemaphoreType.DMA((2 * nbuf + 6 + ncut,)),
            ],
            compiler_params=pltpu.CompilerParams(
                vmem_limit_bytes=100 * 2**20, flags=flags,
                disable_bounds_checks=not bounds, disable_semaphore_checks=not sem_checks),
        )(A_x, kt, vt, wq, wo, B_w_r, wg, wu, wd)
    return fn


pallas_sequential_preLN__sliding_block_cached__moe_arch_mod__decode_kernel = jax.jit(make())
```

```python
import jax
import jax.numpy as jnp
from jax import lax
import jax.experimental.pallas as pl
import jax.experimental.pallas.tpu as pltpu

EPS = 1e-5
LANES = 128
RUN = 512
GROUP_TILES = 256
LAG = 26
LOOK = 2
NBUF = 4
FFN_GROUPS = 4
DOWN_CUTS = (0, 128, 256, 384)
LAST_CUTS = (128, 256, 320, 352, 384)

K_, V_, Q_, O_, G_, U_, D_ = range(7)
SEM_K, SEM_V = 0, NBUF
SEM_Q, SEM_O, SEM_G, SEM_U, SEM_X, SEM_R, SEM_DOWN = range(2 * NBUF, 2 * NBUF + 7)
SEM_LAST = SEM_DOWN + len(DOWN_CUTS) - 1
NUM_SEMS = SEM_LAST + len(LAST_CUTS) - 1


def _copy_stream(H, Dh, W, D, F, proj_groups):
    def sweep(a, groups, step, col, head=None):
        return [((a, g, 1, col, head), (a, g + 1, step - 1, col, head))
                for g in range(0, groups, step)]

    first = [p for c in range(GROUP_TILES * LANES // RUN) for p in sweep(Q_, proj_groups, 5, c)]
    pairs = list(first)
    for h in range(H):
        for a in (K_, V_):
            for c in range(W // RUN):
                pairs += sweep(a, Dh // 8, 6, c, h)
    for c in range(GROUP_TILES * LANES // RUN):
        pairs += sweep(O_, proj_groups, 5, c)
    last = FFN_GROUPS - 1
    for c in range(D // FFN_GROUPS // 8 * (F // RUN)):
        pairs += sweep(G_, FFN_GROUPS, FFN_GROUPS, c)
        pairs += [((U_, last, 1, c, None), (U_, 0, last, c, None))]
    for c in range(F // FFN_GROUPS // 8):
        if 8 * c < LAST_CUTS[0]:
            pairs += sweep(D_, FFN_GROUPS, FFN_GROUPS, c)
        else:
            pairs += [((D_, 0, last, c, None), (D_, last, 1, c, None))]

    stream = [(b, 1) for _, b in pairs[:LAG]]
    for j, (a, _) in enumerate(pairs):
        stream.append((a, 0))
        if j + LAG < len(pairs):
            stream.append((pairs[j + LAG][1], 1))
    per_head = 2 * 2 * (W // RUN) * (Dh // 8 // 6)
    return stream, LAG + 2 * len(first), per_head


def _part(items, i, n):
    return items[len(items) * i // n:len(items) * (i + 1) // n]


def _layernorm(x):
    m = jnp.mean(x, axis=-1, keepdims=True)
    d = x - m
    v = jnp.mean(d * d, axis=-1, keepdims=True)
    return d / jnp.sqrt(v + EPS)


def _kernel(x_hbm, kt_hbm, vt_hbm, wq_hbm, wo_hbm, wr_hbm, wg_hbm, wu_hbm, wd_hbm,
            o_ref,
            x_s, wr_s, wq_s, wo_s, wg_s, wu_s, wd_s, k_s, v_s, q_s, p_s, o_s, sems):
    _, H, Dh, Sk = kt_hbm.shape
    W = k_s.shape[-1]
    D = x_hbm.shape[-1]
    F = wg_hbm.shape[-1]
    f32, bf16 = jnp.float32, jnp.bfloat16
    last = FFN_GROUPS - 1

    def start(copy, queue, i):
        a, g, ng, c, head = copy
        if a in (K_, V_):
            hbm, buf, sem = (kt_hbm, k_s, SEM_K) if a == K_ else (vt_hbm, v_s, SEM_V)
            h = head + i
            slot = h & (NBUF - 1)
            rows = pl.ds(8 * g, 8 * ng)
            src = hbm.at[0, h, rows, pl.ds(Sk - W + RUN * c, RUN)]
            dst = buf.at[slot, rows, pl.ds(RUN * c, RUN)]
            sem = sem + slot
        else:
            if a in (Q_, O_):
                hbm, buf, sem = (wq_hbm, wq_s, SEM_Q) if a == Q_ else (wo_hbm, wo_s, SEM_O)
                idx = (pl.ds(g, ng), pl.ds(c * RUN // LANES, RUN // LANES))
            elif a in (G_, U_):
                hbm, buf, sem = (wg_hbm, wg_s, SEM_G) if a == G_ else (wu_hbm, wu_s, SEM_U)
                r, col = divmod(c, F // RUN)
                idx = (pl.ds(g, ng), pl.ds(8 * r, 8), pl.ds(RUN * col, RUN))
            else:
                hbm, buf = wd_hbm, wd_s
                idx = (pl.ds(g, ng), pl.ds(8 * c, 8))
                cuts, sem = DOWN_CUTS, SEM_DOWN
                if g == last and 8 * c >= LAST_CUTS[0]:
                    cuts, sem = LAST_CUTS, SEM_LAST
                sem += sum(cut <= 8 * c for cut in cuts[1:])
            src, dst = hbm.at[idx], buf.at[idx]
        pltpu.make_async_copy(src, dst, sems.at[sem]).start(priority=queue)

    def issue(copies, i=0):
        for copy, queue in copies:
            start(copy, queue, i)

    def done(dst, sem):
        pltpu.make_async_copy(dst, dst, sems.at[sem]).wait()

    def slab(ref, width, r0, r1, c0, c1):
        def tile(i, j):
            n = i * (width // LANES) + j
            return ref[n // GROUP_TILES, n % GROUP_TILES]
        return jnp.concatenate(
            [jnp.concatenate([tile(i, j) for i in range(r0 // 8, r1 // 8)], axis=0)
             for j in range(c0 // LANES, c1 // LANES)], axis=1)

    stream, head0, per_head = _copy_stream(H, Dh, W, D, F, wq_hbm.shape[0])
    n_loop = H - LOOK - 1
    x_cp = pltpu.make_async_copy(x_hbm, x_s, sems.at[SEM_X])
    wr_cp = pltpu.make_async_copy(wr_hbm, wr_s, sems.at[SEM_R])

    issue(stream[:LAG + 14])
    x_cp.start()
    wr_cp.start(priority=1)
    issue(stream[LAG + 14:head0 + (LOOK - 1) * per_head])
    x_cp.wait()
    x = x_s[0].astype(f32)
    xn = jnp.broadcast_to(_layernorm(x), (8, D)).astype(bf16)
    done(wq_s, SEM_Q)
    copies = stream[head0 + (LOOK - 1) * per_head:head0 + LOOK * per_head]
    for c in range(H // 2):
        issue(_part(copies, c, H // 2))
        w = slab(wq_s, H * Dh, 0, D, 2 * c * Dh, 2 * (c + 1) * Dh)
        q2 = jnp.dot(xn, w, preferred_element_type=f32)
        q_s[2 * c] = q2[:, :Dh]
        q_s[2 * c + 1] = q2[:, Dh:]

    def head(h, copies, i=0):
        parts = Dh // 16 + 2
        slot = h & (NBUF - 1)
        done(k_s.at[slot], SEM_K + slot)
        issue(_part(copies, 0, parts), i)
        s = jnp.dot(q_s[h].astype(bf16), k_s[slot], preferred_element_type=f32) * Dh ** -0.5
        issue(_part(copies, 1, parts), i)
        m = jnp.max(s, axis=-1, keepdims=True)
        e = jnp.exp(s - m)
        inv = 1.0 / jnp.sum(e, axis=-1, keepdims=True)
        p_s[...] = e
        done(v_s.at[slot], SEM_V + slot)
        acc = []
        for r in range(Dh // 16):
            issue(_part(copies, r + 2, parts), i)
            a0 = jnp.zeros((8, LANES), f32)
            a1 = jnp.zeros((8, LANES), f32)
            for j in range(W // LANES):
                cols = slice(j * LANES, (j + 1) * LANES)
                vv = v_s[slot, r * 16:(r + 1) * 16, cols].astype(f32)
                pp = p_s[:, cols]
                a0 = a0 + vv[:8] * pp
                a1 = a1 + vv[8:] * pp
            acc += [a0, a1]
        acc.append(jnp.zeros((o_s.shape[-1] - Dh, LANES), f32))
        o_s[h] = jnp.sum(jnp.concatenate(acc, axis=0).T, axis=0, keepdims=True) * inv

    copies = stream[head0 + LOOK * per_head:head0 + (LOOK + 1) * per_head]
    lax.fori_loop(0, n_loop, lambda h, _: head(h, copies, h), None)

    tail = stream[head0 + (LOOK + n_loop) * per_head:]
    n0 = max(i for i, (copy, _) in enumerate(tail) if copy[0] == O_) + 84
    n1, n2 = n0 + 72, len(tail) - 24
    for t in range(LOOK + 1):
        head(n_loop + t, _part(tail[:n0], t, LOOK + 1))

    done(wo_s, SEM_O)
    attn = jnp.zeros((8, D), f32)
    for h in range(H):
        issue(_part(tail[n0:n1], h, H))
        w = slab(wo_s, D, h * Dh, (h + 1) * Dh, 0, D)
        attn = attn + jnp.dot(o_s[h][:, :Dh].astype(bf16), w, preferred_element_type=f32)
    hres = x + attn[:1]
    hn = _layernorm(hres)
    wr_cp.wait()
    wr = wr_s[...].astype(f32).reshape(1, D)
    gate = jax.nn.sigmoid(jnp.sum(hn * wr, axis=-1, keepdims=True))
    hb = jnp.broadcast_to(hn, (8, D)).astype(bf16)

    issue(tail[n1:n2])
    done(wg_s, SEM_G)
    issue(tail[n2:])
    g = jnp.dot(hb, wg_s[...].reshape(D, F), preferred_element_type=f32)
    done(wu_s, SEM_U)
    u = jnp.dot(hb, wu_s[...].reshape(D, F), preferred_element_type=f32)
    gu = (g * jax.nn.sigmoid(g) * u).astype(bf16)
    rows = F // FFN_GROUPS
    r0 = LAST_CUTS[0]
    gcol = jnp.broadcast_to(gu[:1, last * rows + r0:].astype(f32), (LANES, rows - r0)).T
    base = hres + hn

    y = jnp.zeros((8, D), f32)
    for c, (lo, hi) in enumerate(zip(DOWN_CUTS, DOWN_CUTS[1:])):
        ng = FFN_GROUPS if lo < r0 else last
        lhs = jnp.concatenate([gu[:, i * rows + lo:i * rows + hi] for i in range(ng)], axis=1)
        done(wd_s.at[pl.ds(0, ng), pl.ds(lo, hi - lo)], SEM_DOWN + c)
        w = wd_s[:ng, lo:hi, :].reshape(ng * (hi - lo), D)
        y = y + jnp.dot(lhs, w, preferred_element_type=f32)
    z = jnp.zeros((8, D), f32)
    for c, (lo, hi) in enumerate(zip(LAST_CUTS, LAST_CUTS[1:])):
        done(wd_s.at[last, pl.ds(lo, hi - lo)], SEM_LAST + c)
        for r in range(lo, hi, 8):
            gk = jnp.concatenate([gcol[r - r0:r - r0 + 8]] * (D // LANES), axis=1)
            z = z + wd_s[last, r:r + 8, :].astype(f32) * gk
    out = base + (y[:1] + jnp.sum(z, axis=0, keepdims=True)) * gate
    o_ref[0] = out.astype(o_ref.dtype)


@jax.jit
def pallas_sequential_preLN__sliding_block_cached__moe_arch_mod__decode_kernel(
    A_x: jax.Array,
    A_k_cache: jax.Array,
    A_v_cache: jax.Array,
    A_wq: jax.Array,
    A_wo: jax.Array,
    B_x: jax.Array,
    B_w_r: jax.Array,
    B_w_gate: jax.Array,
    B_w_up: jax.Array,
    B_w_down: jax.Array,
):
    del B_x
    _, H, Sk, Dh = A_k_cache.shape
    W = min(4096, max(256, Sk // 4))
    assert W % RUN == 0 and Dh % 48 == 0 and A_wq.size % (5 * GROUP_TILES * 8 * LANES) == 0
    assert B_w_down.shape[0] == FFN_GROUPS * DOWN_CUTS[-1] == FFN_GROUPS * LAST_CUTS[-1]

    def tiles(a):
        r, c = a.shape
        t = a.reshape(r // 8, 8, c // LANES, LANES).transpose(0, 2, 1, 3)
        return t.reshape(-1, GROUP_TILES, 8, LANES)

    def groups(a):
        return a.reshape(FFN_GROUPS, a.shape[0] // FFN_GROUPS, a.shape[1])

    kt = jnp.transpose(A_k_cache, (0, 1, 3, 2))
    vt = jnp.transpose(A_v_cache, (0, 1, 3, 2))
    wq, wo = tiles(A_wq), tiles(A_wo)
    wg, wu, wd = groups(B_w_gate), groups(B_w_up), groups(B_w_down)
    like = lambda a: pltpu.VMEM(a.shape, a.dtype)
    return pl.pallas_call(
        _kernel,
        out_shape=jax.ShapeDtypeStruct(A_x.shape, A_x.dtype),
        in_specs=[pl.BlockSpec(memory_space=pl.ANY)] * 9,
        scratch_shapes=[
            like(A_x), like(B_w_r), like(wq), like(wo), like(wg), like(wu), like(wd),
            pltpu.VMEM((NBUF, Dh, W), A_k_cache.dtype),
            pltpu.VMEM((NBUF, Dh, W), A_v_cache.dtype),
            pltpu.VMEM((H, 8, Dh), jnp.float32),
            pltpu.VMEM((8, W), jnp.float32),
            pltpu.VMEM((H, 8, pl.cdiv(Dh, LANES) * LANES), jnp.float32),
            pltpu.SemaphoreType.DMA((NUM_SEMS,)),
        ],
        compiler_params=pltpu.CompilerParams(
            vmem_limit_bytes=64 * 2**20,
            disable_bounds_checks=True,
            disable_semaphore_checks=True,
        ),
    )(A_x, kt, vt, wq, wo, B_w_r, wg, wu, wd)
```
